```python
import os as _os
_os.environ.setdefault("JAX_PLATFORMS", "cpu")
import jax
import jax.numpy as jnp

def _softmax(x, axis=-1):
    return jax.nn.softmax(x, axis=axis)
def _gelu(x):
    return jax.nn.gelu(x, approximate=True)
def _silu(x):
    return jax.nn.silu(x)
def _sigmoid(x):
    return jax.nn.sigmoid(x)
def _layernorm(x, axis=-1, eps=1e-5):
    m = jnp.mean(x, axis=axis, keepdims=True)
    v = jnp.var(x, axis=axis, keepdims=True)
    return (x - m) / jnp.sqrt(v + eps)
def _scatter_add(tgt, idx, src, axis=0):
    return tgt.at[idx].add(src)
def _segment_sum(src, seg, n):
    return jax.ops.segment_sum(src, seg, n)
class _Rng:
    def __init__(self, key):
        self._k = key
    def _next(self):
        self._k, sub = jax.random.split(self._k)
        return sub
    def normal(self, shape):
        return jax.random.normal(self._next(), shape, dtype=jnp.bfloat16)
    def randint(self, lo, hi, shape):
        return jax.random.randint(self._next(), shape, lo, hi, dtype=jnp.int32)
    def uniform(self, shape, lo=0.0, hi=1.0):
        return jax.random.uniform(self._next(), shape, jnp.bfloat16, lo, hi)
    def permutation(self, n):
        return jax.random.permutation(self._next(), n)


kernel_name = 'concat_heads__mha_block_cached__gqa_block_cached__near_ridge'

def setup_inputs():
    _rng = _Rng(jax.random.key(int.from_bytes(__import__("os").urandom(4), "little")))
    _w = (lambda a: (lambda t: t.astype(jnp.bfloat16) if jnp.issubdtype(t.dtype, jnp.floating) else t)(jnp.asarray(a)))
    def _A_setup():
        B, Sq, D = 16, 160, 512
        H, Sk, Dh = 32, 1024, 128
        return {
            "x": _w((lambda *s: _rng.normal(s) * 0.8)(B, Sq, D)),
            "k_cache": _w((lambda *s: _rng.normal(s) * 0.8)(B, H, Sk, Dh)),
            "v_cache": _w((lambda *s: _rng.normal(s) * 0.05)(B, H, Sk, Dh)),
            "wq": _w((lambda *s: _rng.normal(s) * 0.8)(D, H * Dh) * (D ** -0.5)),
            "wo": _w((lambda *s: _rng.normal(s) * 0.05)(H * Dh, D) * ((H * Dh) ** -0.5)),
        }
    _A_in = _A_setup()

    def _B_setup():
        B, Sq, D = 16, 160, 512
        Hq, Hkv, Sk, Dh = 32, 32, 1024, 128
        assert Hq % Hkv == 0, (Hq, Hkv)
        return {
            "x": _w((lambda *s: _rng.normal(s) * 0.8)(B, Sq, D)),
            "k_cache": _w((lambda *s: _rng.normal(s) * 0.8)(B, Hkv, Sk, Dh)),
            "v_cache": _w((lambda *s: _rng.normal(s) * 0.05)(B, Hkv, Sk, Dh)),
            "wq": _w((lambda *s: _rng.normal(s) * 0.8)(D, Hq * Dh) * (D ** -0.5)),
            "wo": _w((lambda *s: _rng.normal(s) * 0.05)(Hq * Dh, D) * ((Hq * Dh) ** -0.5)),
        }
    _B_in = _B_setup()

    return {
        "A_x": _A_in["x"],
        "A_k_cache": _A_in["k_cache"],
        "A_v_cache": _A_in["v_cache"],
        "A_wq": _A_in["wq"],
        "A_wo": _A_in["wo"],
        "B_x": _B_in["x"],
        "B_k_cache": _B_in["k_cache"],
        "B_v_cache": _B_in["v_cache"],
        "B_wq": _B_in["wq"],
        "B_wo": _B_in["wo"],
    }

def reference(A_x, A_k_cache, A_v_cache, A_wq, A_wo, B_x, B_k_cache, B_v_cache, B_wq, B_wo):
    def _A_ref(x, k_cache, v_cache, wq, wo):
        B, Sq, D = x.shape
        H, Dh = 32, 128
        q = (lambda x, *d: x.transpose(*d))((x @ wq).reshape(B, Sq, H, Dh), 0, 2, 1, 3)
        scores = jnp.einsum("bhqd,bhkd->bhqk", q, k_cache) * (Dh ** -0.5)
        p = _softmax(scores, axis=-1)
        o = jnp.einsum("bhqk,bhkd->bhqd", p, v_cache)
        return (lambda x, *d: x.transpose(*d))(o, 0, 2, 1, 3).reshape(B, Sq, H * Dh) @ wo

    def _B_ref(x, k_cache, v_cache, wq, wo):
        B, Sq, D = x.shape
        Hq, Dh = 32, 128
        Hkv = k_cache.shape[1]
        rep = Hq // Hkv
        q = (lambda x, *d: x.transpose(*d))((x @ wq).reshape(B, Sq, Hq, Dh), 0, 2, 1, 3)
        k = jnp.repeat(k_cache, rep, axis=1)
        v = jnp.repeat(v_cache, rep, axis=1)
        scores = jnp.einsum("bhqd,bhkd->bhqk", q, k) * (Dh ** -0.5)
        p = _softmax(scores, axis=-1)
        o = jnp.einsum("bhqk,bhkd->bhqd", p, v)
        return (lambda x, *d: x.transpose(*d))(o, 0, 2, 1, 3).reshape(B, Sq, Hq * Dh) @ wo

    a = _A_ref(A_x, A_k_cache, A_v_cache, A_wq, A_wo)
    b = _B_ref(B_x, B_k_cache, B_v_cache, B_wq, B_wo)
    return jnp.concatenate([a, b], axis=-1)
```

```python
import functools, math
import jax, jax.numpy as jnp
from jax import lax
from jax.experimental import pallas as pl
from jax.experimental.pallas import tpu as pltpu

B, Sq, D, H, Sk, Dh = 16, 160, 512, 32, 1024, 128
C = Dh ** -0.5 * math.log2(math.e)
NT = (((1,), (1,)), ((), ()))
f32, bf16 = jnp.float32, jnp.bfloat16

def make(P=4, LP=2, nr=128, prio=(1, 1, 1, 0), dma=True, compute=True, flags=None, recip='exact', nbc=True):
    G = H // P
    NIT = B * G
    npc = Sk // nr

    def kern(ax, ak, av, awq, awo, bx, bk, bv, bwq, bwo, out, *scr):
        scr = list(scr)
        kb = [[scr.pop(0) for _ in range(P)] for _ in range(2)]
        vb = [[scr.pop(0) for _ in range(P)] for _ in range(2)]
        wq = [scr.pop(0) for _ in range(2)]
        wo = [scr.pop(0) for _ in range(2)]
        xb = [scr.pop(0) for _ in range(2)]
        acc = [scr.pop(0) for _ in range(2)]
        ob = scr.pop(0)
        qs, os_ = scr.pop(0), scr.pop(0)
        ksem, vsem, wsem, xsem, osem = scr
        xh, kh, vh, wqh, woh = (ax, bx), (ak, bk), (av, bv), (awq, bwq), (awo, bwo)

        def pieces(pair, u):
            res = []
            for r in range(npc):
                rs = pl.ds(r * nr, nr)
                for s in range(2):
                    res.append(pltpu.make_async_copy(kh[s].at[pair, rs], kb[s][u].at[rs], ksem.at[s, u]))
                    res.append(pltpu.make_async_copy(vh[s].at[pair, rs], vb[s][u].at[rs], vsem.at[s, u]))
            return [(c, prio[i % len(prio)]) for i, c in enumerate(res)]
        def kwait(s, u):
            if dma: pltpu.make_async_copy(kb[s][u], kb[s][u], ksem.at[s, u]).wait()
        def vwait(s, u):
            if dma: pltpu.make_async_copy(vb[s][u], vb[s][u], vsem.at[s, u]).wait()
        def xcopy(s, b):
            return pltpu.make_async_copy(xh[s].at[b], xb[s].at[b % 2], xsem.at[s])
        def ocopy(b):
            return pltpu.make_async_copy(ob, out.at[b], osem.at[0])

        def qproj(s, xslot, g, u):
            q = jnp.dot(xb[s][xslot], wq[s][g, :, u * Dh:(u + 1) * Dh], preferred_element_type=f32)
            return (q * C).astype(bf16)
        def oproj(s, o, g, u):
            return jnp.dot(o, wo[s][g, u * Dh:(u + 1) * Dh, :], preferred_element_type=f32)

        for s in range(2):
            xcopy(s, 0).start()
        wc = []
        for g in range(G):
            for s in range(2):
                wc.append(pltpu.make_async_copy(wqh[s].at[:, pl.ds(g * P * Dh, P * Dh)], wq[s].at[g], wsem.at[0]))
                wc.append(pltpu.make_async_copy(woh[s].at[pl.ds(g * P * Dh, P * Dh)], wo[s].at[g], wsem.at[0]))
        for i, c in enumerate(wc): c.start(priority=i % 2)
        if dma:
            for u in range(LP):
                for c, p in pieces(u, u): c.start(priority=p)
        for s in range(2):
            xcopy(s, 0).wait()
            acc[s][...] = jnp.zeros_like(acc[s])
        os_[...] = jnp.zeros_like(os_)
        for c in wc: c.wait()
        qs[...] = qproj(0, 0, 0, 0)

        def body(it, last):
            b = it // G
            g = it % G
            gp = (it + G - 1) % G
            itn = jnp.minimum(it + 1, NIT - 1)
            q = qs[...]
            o = os_[...]
            for u in range(P):
                if dma and not (last and u + LP >= P):
                    pcs = pieces(it * P + u + LP, (u + LP) % P)
                else:
                    pcs = []
                nph = 12
                ph = [0]
                def issue(n):
                    lo = len(pcs) * ph[0] // nph; ph[0] += n; hi = len(pcs) * ph[0] // nph
                    for c, p in pcs[lo:hi]: c.start(priority=p)
                for s in range(2):
                    kwait(s, u)
                    issue(2)
                    if compute:
                        sc = lax.dot_general(q, kb[s][u][...], NT, preferred_element_type=f32)
                    issue(1)
                    if s == 1 and u == P - 1 and not last:
                        @pl.when(g == G - 1)
                        def _():
                            for s2 in range(2): xcopy(s2, b + 1).wait()
                    if compute:
                        if s == 0:
                            q = qproj(1, b % 2, g, u)
                        elif u < P - 1:
                            q = qproj(0, b % 2, g, u + 1)
                        elif not last:
                            q = qproj(0, (itn // G) % 2, itn % G, 0)
                    issue(1)
                    if compute:
                        if s == 1:
                            a = acc[0][...]
                            if u == 0: a = jnp.where(g == 0, 0.0, a)
                            a = a + oproj(0, o, g, u)
                            acc[0][...] = a
                            if u == P - 1:
                                ob[:, :D] = a.astype(bf16)
                        elif u > 0:
                            a = acc[1][...]
                            if u == 1: a = jnp.where(g == 0, 0.0, a)
                            acc[1][...] = a + oproj(1, o, g, u - 1)
                        else:
                            a = acc[1][...] + oproj(1, o, gp, P - 1)
                            acc[1][...] = a
                            ob[:, D:] = a.astype(bf16)
                    if s == 0 and u == 0 and not last:
                        @pl.when(jnp.logical_and(g == 0, b > 0))
                        def _():
                            ocopy(b - 1).start()
                        @pl.when(jnp.logical_and(g == 0, b < B - 1))
                        def _():
                            for s2 in range(2): xcopy(s2, b + 1).start()
                    if s == 0 and u == P - 1 and not last:
                        @pl.when(jnp.logical_and(g == 0, b > 0))
                        def _():
                            ocopy(b - 1).wait()
                    vwait(s, u)
                    issue(2)
                    if compute:
                        m = jnp.max(sc, axis=-1, keepdims=True)
                        p = jnp.exp2(sc - m)
                        l = jnp.sum(p, axis=-1, keepdims=True)
                        pv = jnp.dot(p.astype(bf16), vb[s][u][...], preferred_element_type=f32)
                        r = 1.0 / l if recip == 'exact' else pltpu.reciprocal(l, approx=True)
                        o = (pv * r).astype(bf16)
            if not last:
                qs[...] = q
                os_[...] = o
            return o
        def loop_body(it, c):
            body(it, False)
            return c
        lax.fori_loop(0, NIT - 1, loop_body, 0)
        o = body(NIT - 1, True)
        a = acc[1][...] + oproj(1, o, G - 1, P - 1)
        ob[:, D:] = a.astype(bf16)
        c = ocopy(B - 1); c.start(); c.wait()

    def f(ax, ak, av, awq, awo, bx, bk, bv, bwq, bwo):
        r = lambda t: t.reshape(B * H, Sk, Dh)
        V = pltpu.VMEM
        return pl.pallas_call(kern,
            in_specs=[pl.BlockSpec(memory_space=pl.ANY)] * 10,
            out_specs=pl.BlockSpec(memory_space=pl.ANY),
            out_shape=jax.ShapeDtypeStruct((B, Sq, 2 * D), bf16),
            scratch_shapes=[V((Sk, Dh), bf16)] * (4 * P) + [V((G, D, P * Dh), bf16)] * 2 + [V((G, P * Dh, D), bf16)] * 2
              + [V((2, Sq, D), bf16)] * 2 + [V((Sq, D), f32)] * 2 + [V((Sq, 2 * D), bf16)] + [V((Sq, Dh), bf16)] * 2
              + [pltpu.SemaphoreType.DMA((2, P))] * 2 + [pltpu.SemaphoreType.DMA((1,)), pltpu.SemaphoreType.DMA((2,)), pltpu.SemaphoreType.DMA((1,))],
            compiler_params=pltpu.CompilerParams(vmem_limit_bytes=100 * 2**20, flags=flags, disable_bounds_checks=nbc),
            name='k1',
        )(ax, r(ak), r(av), awq, awo, bx, r(bk), r(bv), bwq, bwo)
    return f


_f = make(4, LP=3, nr=64, flags={"XLA_TPU_RESCHEDULE_DMA_DONES": True})


@jax.jit
def pallas_concat_heads__mha_block_cached__gqa_block_cached__near_ridge_kernel(
    A_x, A_k_cache, A_v_cache, A_wq, A_wo, B_x, B_k_cache, B_v_cache, B_wq, B_wo
):
    return _f(A_x, A_k_cache, A_v_cache, A_wq, A_wo, B_x, B_k_cache, B_v_cache, B_wq, B_wo)
```

```python
import contextlib, functools, math
import jax, jax.numpy as jnp
from jax import lax
from jax.experimental import pallas as pl
from jax.experimental.pallas import tpu as pltpu

B, Sq, D, H, Sk, Dh = 16, 160, 512, 32, 1024, 128
C = Dh ** -0.5 * math.log2(math.e)
NT = (((1,), (1,)), ((), ()))
f32, bf16 = jnp.float32, jnp.bfloat16
T = 128
NTL = Sk // T
HK = Sk // 2
F = {"XLA_TPU_RESCHEDULE_DMA_DONES": True}

PATS = {
    'f2': '0 1 2 3! 4 5 6 7!',
    'f3': '0 1 2! 3 4 5! 6 7!',
    'h4': '0 1 3:64! 2 3:64! 4 5 7:64! 6 7:64!',
    'q4': '0 1 7:32! 2 3 7:32! 4 5 7:32! 6 7:32!',
    'h2': '0 1 2 7:64! 3 4 5 6 7:64!',
}

def make(U=4, LA=18, bb=1, pat='f2', dma=True, flags=F, orows=32, t0=180, peel=True, scopes=False, wpad=128, u32=False, ow0=0, xpad=0, qfirst=True, init_at=4, emit=0):
    G = H // U
    NB = B // 2
    NIT = NB * G
    NR = NTL * U
    lg = G.bit_length() - 1
    SB = 1 << bb
    plan = []
    for u in range(U):
        for r in range(NTL):
            pos = [0] * 8; ops = []
            for t in PATS.get(pat, pat).split():
                st = int(t[0]); p = 0 if t.endswith('!') else 1
                nr = int(t.rstrip('!')[2:] or T)
                ops.append((u, (st // 2) % 2, st // 4, st % 2, r * T + pos[st], nr, p)); pos[st] += nr
            assert pos == [T] * 8
            plan.append(ops)
    sc = jax.named_scope if scopes else (lambda n: contextlib.nullcontext())

    def kern(ax, ak, av, awq, awo, bx, bk, bv, bwq, bwo, out, *scr):
        scr = list(scr)
        kvb = [[[[scr.pop(0) for _ in range(2)] for _ in range(2)] for _ in range(2)] for _ in range(U)]
        wq = [scr.pop(0) for _ in range(2)]
        wo = [scr.pop(0) for _ in range(2)]
        xb = [scr.pop(0) for _ in range(2)]
        acc = [scr.pop(0) for _ in range(2)]
        ob, qs, os_, sem = scr
        xh, kvh, wqh, woh = (ax, bx), ((ak, av), (bk, bv)), (awq, bwq), (awo, bwo)
        osem = sem.at[U, 0, 1, 1]

        def batch(it):
            c = it >> lg
            return (c & (SB - 1)) + ((c >> bb) << (bb + 1))
        def start(it, op):
            u, s, j, kv, r0, nr, p = op
            src = kvh[s][kv].at[pl.ds(batch(it) * H + (it & (G - 1)) * U, SB * H + U)]
            pltpu.make_async_copy(src.at[j * SB * H + u, pl.ds(r0, nr)], kvb[u][s][j][kv].at[pl.ds(r0, nr)], sem.at[u, s, j, kv]).start(priority=p)
        def wait(u, s, j, kv):
            if dma:
                dst = kvb[u][s][j][kv]
                pltpu.make_async_copy(dst, dst, sem.at[u, s, j, kv]).wait()
        def ld(u, s, j, kv, h):
            ref = kvb[u][s][j][kv]
            if u32: return pltpu.bitcast(ref.bitcast(jnp.uint32)[h * HK // 2:(h + 1) * HK // 2, :], bf16)
            return ref[h * HK:(h + 1) * HK, :]
        def qproj(it, u, s, j):
            x = xb[s].at[pl.ds(batch(it), SB + 1)][j * SB, :, :D]
            w = wq[s].at[:, pl.ds(pl.multiple_of((it & (G - 1)) * (U * Dh), U * Dh), U * Dh)][:, u * Dh:(u + 1) * Dh]
            return jnp.dot(x, w, preferred_element_type=f32)
        def oproj(it, u, s, j, o):
            w = wo[s].at[pl.ds(pl.multiple_of((it & (G - 1)) * (U * Dh), U * Dh), U * Dh)][u * Dh:(u + 1) * Dh, :]
            a = acc[s][j]
            if u == 0: a = jnp.where((it & (G - 1)) == 0, 0.0, a)
            a = a + jnp.dot(o, w, preferred_element_type=f32)
            if u == U - 1 and emit == 0:
                ob[batch(it) + j * SB, :, s * D:(s + 1) * D] = a.astype(bf16)
            acc[s][j] = a
            return a
        def emit_out(it, s, j):
            ob[batch(it) + j * SB, :, s * D:(s + 1) * D] = acc[s][j].astype(bf16)
        items = [(u, s, j) for u in range(U) for j in range(2) for s in range(2)]

        def wbody(i, c_):
            for half in range(2):
                j = i + half * 64
                r = pl.ds(pl.multiple_of((j >> 1) * 8, 8), 8); c = pl.ds(pl.multiple_of((j & 1) * 2048, 2048), 2048)
                r2 = pl.ds(pl.multiple_of(j * 32, 32), 32)
                for s in range(2):
                    pltpu.make_async_copy(wqh[s].at[r, c], wq[s].at[r, c], sem.at[U, s, 0, 0]).start(priority=1)
                    pltpu.make_async_copy(woh[s].at[r2], wo[s].at[r2], sem.at[U, s, 0, 1]).start(priority=1 - s)
            return c_
        def xbody(i, c_):
            for r in range(Sq // 32):
                for k in range(4):
                    for s in range(2):
                        pltpu.make_async_copy(xh[s].at[i + 4 * k, pl.ds(r * 32, 32)], xb[s].at[i + 4 * k, pl.ds(r * 32, 32), pl.ds(0, D)], sem.at[U, s, 1, 0]).start(priority=int(not (s and k % 2)))
            return c_
        with sc('S_weights'):
            lax.fori_loop(0, 64, wbody, 0)
        with sc('S_x'):
            lax.fori_loop(0, B // 4, xbody, 0)
        def init():
            for s in range(2):
                acc[s][...] = jnp.zeros_like(acc[s])
                pltpu.make_async_copy(wqh[s], wq[s].at[:, pl.ds(0, H * Dh)], sem.at[U, s, 0, 0]).wait()
                pltpu.make_async_copy(woh[s], wo[s], sem.at[U, s, 0, 1]).wait()
                pltpu.make_async_copy(xh[s], xb[s].at[:, :, pl.ds(0, D)], sem.at[U, s, 1, 0]).wait()
            os_[...] = jnp.zeros_like(os_)
            qs[...] = (qproj(0, *items[0]) * C).astype(bf16)
        for n in range(LA):
            if n == init_at: init()
            if dma:
                for op in plan[n]: start(0, op)
        if init_at >= LA: init()

        early = [b for b in range(B) if b not in (B - 1 - SB, B - 1)]
        runs = [(0, B - 1 - SB)] + ([(B - SB, SB - 1)] if SB > 1 else [])
        def flush_out():
            for j in range(ow0 * 16 // orows, Sq // orows):
                for b0, nb in runs:
                    sl = (pl.ds(b0, nb), pl.ds(j * orows, orows))
                    pltpu.make_async_copy(ob.at[sl], out.at[sl], osem).start(priority=1)

        def body(it, last):
            itp = jnp.maximum(it - 1, 0)
            itn = it + 1 if peel else jnp.minimum(it + 1, NIT - 1)
            q = qs[...]
            o = os_[...]
            small = [(b, r) for r in range(ow0) for b in early]
            for item, (u, s, j) in enumerate(items):
                ops = [(n, op) for n in (2 * item + LA, 2 * item + LA + 1) for op in plan[n % NR]]
                n0 = sum(op[6] == 0 for _, op in ops)
                k = 0; timed = []
                for n, op in ops:
                    timed.append((min(959, t0 * 4 // n0 + k * 960 // n0), n, op))
                    k += op[6] == 0
                    tgt = (n // NR) * 4 * U + items.index(op[:3])
                    assert item + 1 < tgt < item + 4 * U, (item, tgt)
                def issue(ph, val):
                    if not dma: return
                    for t, n, op in timed:
                        if t // 160 != ph: continue
                        u2, s2, j2, kv2, r0, nr, p = op
                        i0 = (t % 160) // 16 * 16
                        if last and n >= NR:
                            if p == 0 and small:
                                b, r = small.pop(0)
                                pltpu.make_async_copy(ob.at[b, pl.ds(16 * r, 16)], out.at[b, pl.ds(16 * r, 16)], osem).start(priority=0)
                            continue
                        if p == 0:
                            kvb[u2][s2][j2][kv2][r0:r0 + 16, :] = val[i0:i0 + 16, :T].astype(bf16)
                        if n < NR: start(it, op)
                        elif peel: start(itn, op)
                        else: pl.when(it < NIT - 1)(functools.partial(start, itn, op))
                def next_q():
                    if item + 1 < len(items): return qproj(it, *items[item + 1])
                    return None if last else qproj(itn, *items[0])
                qk = lambda h: lax.dot_general(q, ld(u, s, j, 0, h), NT, preferred_element_type=f32)
                if item == 0: wait(u, s, j, 0)
                if 2 * item + LA - 2 < NR <= 2 * item + LA:
                    if last: flush_out()
                    elif not peel: pl.when(it == NIT - 1)(flush_out)
                if item == 0 and qfirst:
                    qn = next_q(); issue(0, qn)
                    s0 = qk(0); issue(1, s0)
                    s1 = qk(1)
                    wait(u, s, j, 1)
                    issue(2, s1)
                else:
                    s0 = qk(0); issue(0, s0)
                    s1 = qk(1)
                    qn = next_q()
                    issue(1, s1)
                    wait(u, s, j, 1)
                    issue(2, qn)
                if qn is not None: q = (qn * C).astype(bf16)
                pi = (it, *items[item - 1]) if item else (itp, *items[-1])
                a = oproj(*pi, o)
                issue(3, a)
                mx = s0[:, :T]
                for i in range(1, 4): mx = jnp.maximum(mx, s0[:, i * T:(i + 1) * T])
                for i in range(4): mx = jnp.maximum(mx, s1[:, i * T:(i + 1) * T])
                m = jnp.max(mx, axis=-1, keepdims=True)
                p0 = jnp.exp2(s0 - m); p1 = jnp.exp2(s1 - m)
                l = jnp.sum(p0 + p1, axis=-1, keepdims=True)
                pv0 = jnp.dot(p0.astype(bf16), ld(u, s, j, 1, 0), preferred_element_type=f32)
                if item + 1 < len(items): wait(*items[item + 1], 0)
                issue(4, pv0)
                pv = pv0 + jnp.dot(p1.astype(bf16), ld(u, s, j, 1, 1), preferred_element_type=f32)
                issue(5, pv)
                if emit and pi[1] == U - 1: emit_out(pi[0], pi[2], pi[3])
                o = (pv * (1.0 / l)).astype(bf16)
            for b, r in (small if last else []):
                pltpu.make_async_copy(ob.at[b, pl.ds(16 * r, 16)], out.at[b, pl.ds(16 * r, 16)], osem).start(priority=1)
            if not last:
                qs[...] = q
                os_[...] = o
            return o
        def step(it, c_):
            with sc('S_iter'):
                body(it, False)
            return c_
        with sc('S_loop'):
            lax.fori_loop(0, NIT - int(peel), step, 0)
        o2 = body(NIT - 1, True) if peel else os_[...]
        oproj(NIT - 1, *items[-1], o2)
        if emit: emit_out(NIT - 1, *items[-1][1:])
        for b in (B - 1 - SB, B - 1):
            pltpu.make_async_copy(ob.at[b], out.at[b], osem).start(priority=1)
        with sc('S_drain'):
            pltpu.make_async_copy(ob, out, osem).wait()

    def f(ax, ak, av, awq, awo, bx, bk, bv, bwq, bwo):
        r = lambda t: t.reshape(B * H, Sk, Dh)
        V = pltpu.VMEM
        return pl.pallas_call(kern,
            in_specs=[pl.BlockSpec(memory_space=pl.ANY)] * 10,
            out_specs=pl.BlockSpec(memory_space=pl.ANY),
            out_shape=jax.ShapeDtypeStruct((B, Sq, 2 * D), bf16),
            scratch_shapes=[V((Sk, Dh), bf16)] * (8 * U) + [V((D, H * Dh + wpad), bf16)] * 2 + [V((H * Dh, D), bf16)] * 2
              + [V((B, Sq, D + xpad), bf16)] * 2 + [V((2, Sq, D), f32)] * 2 + [V((B, Sq, 2 * D), bf16)] + [V((Sq, Dh), bf16)] * 2
              + [pltpu.SemaphoreType.DMA((U + 1, 2, 2, 2))],
            compiler_params=pltpu.CompilerParams(vmem_limit_bytes=100 * 2**20, flags=flags, disable_bounds_checks=True, disable_semaphore_checks=True),
            name='k5',
        )(ax, r(ak), r(av), awq, awo, bx, r(bk), r(bv), bwq, bwo)
    return f

_f = make(emit=1,u32=True,peel=False,U=8,LA=18)


@jax.jit
def pallas_concat_heads__mha_block_cached__gqa_block_cached__near_ridge_kernel(
    A_x, A_k_cache, A_v_cache, A_wq, A_wo, B_x, B_k_cache, B_v_cache, B_wq, B_wo
):
    return _f(A_x, A_k_cache, A_v_cache, A_wq, A_wo, B_x, B_k_cache, B_v_cache, B_wq, B_wo)
```

```python
import functools
import math

import jax
import jax.experimental.pallas as pl
import jax.experimental.pallas.tpu as pltpu
import jax.numpy as jnp
from jax import lax

F32, BF16 = jnp.float32, jnp.bfloat16

LANES = 128
PACKED_ROWS = 16
TILE_ELEMS = 128 * 128
GROUP = 4
HEADS_PER_STEP = 4
ITEMS = HEADS_PER_STEP * 2 * GROUP
PHASES = 6
LOOKAHEAD_ITEMS = 12


def _round_order():
    bulk = [(a, j, 1) for a in (0, 2, 1) for j in range(GROUP)]
    return [t for j in range(GROUP) for t in (*bulk[3 * j : 3 * j + 3], (3, j, 0))]


ROUND = _round_order()


def _item(i):
    return i // (2 * GROUP), i // GROUP % 2, i % GROUP


def _kernel(ax, ak, av, awq, awo, bx, bk, bv, bwq, bwo, out, *scratch):
    x_hbm, wq_hbm, wo_hbm = (ax, bx), (awq, bwq), (awo, bwo)
    kv_hbm = ((ak, av), (bk, bv))
    kv = [scratch[2 * i : 2 * i + 2] for i in range(ITEMS)]
    scratch = scratch[2 * ITEMS :]
    wq, wo, x, acc = (scratch[2 * i : 2 * i + 2] for i in range(4))
    out_buf, q_carry, o_carry, sem = scratch[8:]
    wq_sem, wo_sem, x_sem, out_sem = range(ITEMS, ITEMS + 4)

    batches, sq, d = ax.shape
    _, sk, dh = ak.shape
    heads = awq.shape[1] // dh
    steps_per_group = heads // HEADS_PER_STEP
    steps = batches // GROUP * steps_per_group
    half = sk // 2
    q_scale = dh**-0.5 * math.log2(math.e)

    def first_batch(step):
        group = step >> (steps_per_group.bit_length() - 1)
        return (group & 1) + (group >> 1) * 2 * GROUP

    def first_head(step):
        return (step & (steps_per_group - 1)) * HEADS_PER_STEP

    tile_rows = TILE_ELEMS // dh
    rounds = sk // tile_rows
    tiles_per_item = 2 * rounds
    tiles_per_step = ITEMS * tiles_per_item
    stagger = rounds // 2 * len(ROUND)

    def tile(position):
        array, j, queue = ROUND[position % len(ROUND)]
        branch, which = divmod(array, 2)
        ahead, n = divmod(position - branch * stagger, tiles_per_step)
        head, r = divmod(n // len(ROUND), rounds)
        return ahead, (2 * head + branch) * GROUP + j, which, r * tile_rows, queue

    def start_tile(step, i, which, row, queue):
        head, branch, j = _item(i)
        span = 2 * (GROUP - 1) * heads + HEADS_PER_STEP
        first = first_batch(step) * heads + first_head(step)
        src = kv_hbm[branch][which].at[pl.ds(first, span)]
        rows = pl.ds(row, tile_rows)
        pltpu.make_async_copy(
            src.at[2 * j * heads + head, rows], kv[i][which].at[rows], sem.at[i, which]
        ).start(priority=queue)

    def wait_kv(i, which):
        pltpu.make_async_copy(kv[i][which], kv[i][which], sem.at[i, which]).wait()

    def step_heads(step):
        return pl.ds(pl.multiple_of(first_head(step) * dh, dh), HEADS_PER_STEP * dh)

    def q_proj(step, i):
        head, branch, j = _item(i)
        xs = x[branch].at[pl.ds(first_batch(step), 2 * GROUP - 1)][2 * j]
        w = wq[branch].at[:, step_heads(step)][:, head * dh : (head + 1) * dh]
        return jnp.dot(xs, w, preferred_element_type=F32)

    def o_proj(step, i, o):
        head, branch, j = _item(i)
        total = acc[branch][j]
        if head == 0:
            total = jnp.where(first_head(step) == 0, 0.0, total)
        w = wo[branch].at[step_heads(step)][head * dh : (head + 1) * dh, :]
        total = total + jnp.dot(o, w, preferred_element_type=F32)
        acc[branch][j] = total
        return total

    def stage_output(step, i):
        head, branch, j = _item(i)
        if head == HEADS_PER_STEP - 1:
            b = first_batch(step) + 2 * j
            rows = pl.ds(pl.multiple_of((b & 1) * sq, sq), sq)
            out_buf[b >> 1, rows, pl.ds(branch * d, d)] = acc[branch][j].astype(BF16)

    def write_output(first_pair, pairs, row):
        block = (pl.ds(first_pair, pairs), pl.ds(row, PACKED_ROWS))
        pltpu.make_async_copy(
            out_buf.at[block], out.at[block], sem.at[out_sem, 0]
        ).start(priority=1)

    pairs = batches // 2
    late_pair = pairs - GROUP
    early_writes = [(0, pairs, r) for r in range(0, sq, PACKED_ROWS)]
    if late_pair:
        early_writes += [(0, late_pair, r) for r in range(sq, 2 * sq, PACKED_ROWS)]
    late_writes = [(late_pair, GROUP, r) for r in range(sq, 2 * sq, PACKED_ROWS)]

    wq_cols = min(heads * dh, TILE_ELEMS // 8)
    wq_rows = TILE_ELEMS // wq_cols
    wq_tiles_per_row = heads * dh // wq_cols
    d_rows = TILE_ELEMS // d
    weight_rounds = heads * dh * d // TILE_ELEMS // GROUP

    @pl.loop(0, weight_rounds)
    def _(n):
        for array, j, queue in ROUND:
            branch, which = divmod(array, 2)
            t = n + j * weight_rounds
            if which == 0:
                r = (t >> (wq_tiles_per_row.bit_length() - 1)) * wq_rows
                c = (t & (wq_tiles_per_row - 1)) * wq_cols
                block = (
                    pl.ds(pl.multiple_of(r, wq_rows), wq_rows),
                    pl.ds(pl.multiple_of(c, wq_cols), wq_cols),
                )
                src, dst, s = wq_hbm[branch], wq[branch], wq_sem
            else:
                block = pl.ds(pl.multiple_of(t * d_rows, d_rows), d_rows)
                src, dst, s = wo_hbm[branch], wo[branch], wo_sem
            pltpu.make_async_copy(
                src.at[block], dst.at[block], sem.at[s, branch]
            ).start(priority=queue)

    x_rounds = batches // (2 * GROUP)

    @pl.loop(0, x_rounds)
    def _(n):
        for row in range(0, sq, d_rows):
            for array, j, queue in ROUND:
                branch, which = divmod(array, 2)
                block = (n + (2 * j + which) * x_rounds, pl.ds(row, d_rows))
                pltpu.make_async_copy(
                    x_hbm[branch].at[block], x[branch].at[block], sem.at[x_sem, branch]
                ).start(priority=queue)

    lookahead = LOOKAHEAD_ITEMS * tiles_per_item
    for position in range(lookahead):
        if position == lookahead // 2:
            for branch in range(2):
                acc[branch][...] = jnp.zeros_like(acc[branch])
                wq_dst = wq[branch].at[:, pl.ds(0, heads * dh)]
                for src, dst, s in (
                    (wq_hbm, wq_dst, wq_sem),
                    (wo_hbm, wo[branch], wo_sem),
                    (x_hbm, x[branch], x_sem),
                ):
                    pltpu.make_async_copy(src[branch], dst, sem.at[s, branch]).wait()
            o_carry[...] = jnp.zeros_like(o_carry)
            q_carry[...] = (q_proj(0, 0) * q_scale).astype(BF16)
        ahead, *t = tile(position)
        if ahead == 0:
            start_tile(0, *t)

    @pl.loop(0, steps)
    def _(step):
        prev_step = jnp.maximum(step - 1, 0)
        next_step = jnp.minimum(step + 1, steps - 1)
        last = step == steps - 1
        writes = list(early_writes)
        q, o = q_carry[...], o_carry[...]

        for i in range(ITEMS):

            def request(phase, result):
                for k in range(tiles_per_item):
                    due, due_row = divmod(
                        (k // 4 * 4 + 3) * PHASES * sq // tiles_per_item, sq
                    )
                    if due != phase:
                        continue
                    position = i * tiles_per_item + k + lookahead
                    ahead, slot, which, row, queue = tile(position)
                    assert i + 1 < ahead * ITEMS + slot < i + ITEMS
                    if queue == 0:
                        r = due_row // PACKED_ROWS * PACKED_ROWS
                        kv[slot][which][pl.ds(row, PACKED_ROWS), :] = result[
                            r : r + PACKED_ROWS, :dh
                        ].astype(BF16)
                    if ahead == 0:
                        start_tile(step, slot, which, row, queue)
                        continue
                    pl.when(jnp.logical_not(last))(
                        functools.partial(start_tile, next_step, slot, which, row, queue)
                    )
                    if writes and k % 4 == 0 and position >= tiles_per_step + stagger:
                        pl.when(last)(functools.partial(write_output, *writes.pop(0)))

            def scores(part):
                keys = kv[i][0][part * half : (part + 1) * half, :]
                return lax.dot_general(
                    q, keys, (((1,), (1,)), ((), ())), preferred_element_type=F32
                )

            following = (step, i + 1) if i + 1 < ITEMS else (next_step, 0)
            previous = (step, i - 1) if i else (prev_step, ITEMS - 1)

            if i == 0:
                wait_kv(i, 0)
                q_next = q_proj(*following)
                request(0, q_next)
                s0 = scores(0)
                request(1, s0)
                s1 = scores(1)
                wait_kv(i, 1)
                request(2, s1)
            else:
                s0 = scores(0)
                request(0, s0)
                s1 = scores(1)
                q_next = q_proj(*following)
                request(1, s1)
                wait_kv(i, 1)
                request(2, q_next)
            q = (q_next * q_scale).astype(BF16)
            request(3, o_proj(*previous, o))

            columns = [s[:, c : c + LANES] for s in (s0, s1) for c in range(0, half, LANES)]
            row_max = jnp.max(functools.reduce(jnp.maximum, columns), axis=-1, keepdims=True)
            p0 = jnp.exp2(s0 - row_max)
            p1 = jnp.exp2(s1 - row_max)
            row_sum = jnp.sum(p0 + p1, axis=-1, keepdims=True)

            pv = jnp.dot(p0.astype(BF16), kv[i][1][:half, :], preferred_element_type=F32)
            if i + 1 < ITEMS:
                wait_kv(i + 1, 0)
            request(4, pv)
            pv = pv + jnp.dot(p1.astype(BF16), kv[i][1][half:, :], preferred_element_type=F32)
            request(5, pv)
            stage_output(*previous)
            o = (pv * (1.0 / row_sum)).astype(BF16)

        assert not writes
        q_carry[...] = q
        o_carry[...] = o

    o_proj(steps - 1, ITEMS - 1, o_carry[...])
    stage_output(steps - 1, ITEMS - 1)
    for write in late_writes:
        write_output(*write)
    pltpu.make_async_copy(out_buf, out, sem.at[out_sem, 0]).wait()


@jax.jit
def pallas_concat_heads__mha_block_cached__gqa_block_cached__near_ridge_kernel(
    A_x: jax.Array,
    A_k_cache: jax.Array,
    A_v_cache: jax.Array,
    A_wq: jax.Array,
    A_wo: jax.Array,
    B_x: jax.Array,
    B_k_cache: jax.Array,
    B_v_cache: jax.Array,
    B_wq: jax.Array,
    B_wo: jax.Array,
):
    batches, sq, d = A_x.shape
    _, heads, sk, dh = A_k_cache.shape
    assert B_x.shape == A_x.shape and B_k_cache.shape == A_k_cache.shape
    assert A_wq.shape == B_wq.shape == (d, heads * dh)
    assert batches % (2 * GROUP) == 0
    assert heads >= 2 * HEADS_PER_STEP and heads & (heads - 1) == 0

    def flat(cache):
        return cache.reshape(batches * heads, sk, dh)

    out_shape = (batches // 2, 2 * sq, 2 * d)
    vmem = pltpu.VMEM
    out = pl.pallas_call(
        _kernel,
        in_specs=[pl.BlockSpec(memory_space=pl.ANY)] * 10,
        out_specs=pl.BlockSpec(memory_space=pl.ANY),
        out_shape=jax.ShapeDtypeStruct(out_shape, BF16),
        scratch_shapes=[
            *[vmem((sk, dh), BF16)] * (2 * ITEMS),
            *[vmem((d, heads * dh + LANES), BF16)] * 2,
            *[vmem((heads * dh, d), BF16)] * 2,
            *[vmem((batches, sq, d), BF16)] * 2,
            *[vmem((GROUP, sq, d), F32)] * 2,
            vmem(out_shape, BF16),
            *[vmem((sq, dh), BF16)] * 2,
            pltpu.SemaphoreType.DMA((ITEMS + 4, 2)),
        ],
        compiler_params=pltpu.CompilerParams(
            vmem_limit_bytes=100 * 2**20,
            disable_bounds_checks=True,
            disable_semaphore_checks=True,
            flags={"XLA_TPU_RESCHEDULE_DMA_DONES": True},
        ),
        name="concat_heads_cached_attention",
    )(
        A_x, flat(A_k_cache), flat(A_v_cache), A_wq, A_wo,
        B_x, flat(B_k_cache), flat(B_v_cache), B_wq, B_wo,
    )
    return out.reshape(batches, sq, 2 * d)
```
